```python
import jax
import jax.numpy as jnp

def _softmax(x, axis=-1):
    return jax.nn.softmax(x, axis=axis)

def _gelu(x):
    return jax.nn.gelu(x, approximate=True)

def _silu(x):
    return jax.nn.silu(x)

def _sigmoid(x):
    return jax.nn.sigmoid(x)

def _layernorm(x, axis=-1, eps=1e-05):
    m = jnp.mean(x, axis=axis, keepdims=True)
    v = jnp.var(x, axis=axis, keepdims=True)
    return (x - m) / jnp.sqrt(v + eps)

def _scatter_add(tgt, idx, src, axis=0):
    return tgt.at[idx].add(src)

def _segment_sum(src, seg, n):
    return jax.ops.segment_sum(src, seg, n)

class _Rng:

    def __init__(self, key):
        self._k = key

    def _next(self):
        self._k, sub = jax.random.split(self._k)
        return sub

    def normal(self, shape):
        return jax.random.normal(self._next(), shape, dtype=jnp.bfloat16)

    def randint(self, lo, hi, shape):
        return jax.random.randint(self._next(), shape, lo, hi, dtype=jnp.int32)

    def uniform(self, shape, lo=0.0, hi=1.0):
        return jax.random.uniform(self._next(), shape, jnp.bfloat16, lo, hi)

    def permutation(self, n):
        return jax.random.permutation(self._next(), n)
kernel_name = 'adaLN_cond__sliding_block_cached__mixer_s_mlp__decode'

def setup_inputs():
    _rng = _Rng(jax.random.key(int.from_bytes(__import__("os").urandom(4), "little")))
    _w = lambda a: (lambda t: t.astype(jnp.bfloat16) if jnp.issubdtype(t.dtype, jnp.floating) else t)(jnp.asarray(a))

    def _A_setup():
        B, Sq, D = (1, 1, 448)
        Hq, Hkv, Sk, Dh = (16, 8, 65536, 256)
        assert Hq % Hkv == 0, (Hq, Hkv)
        return {'x': _w((lambda *s: _rng.normal(s) * 0.05)(B, Sq, D)), 'k_cache': _w((lambda *s: _rng.normal(s) * 0.05)(B, Hkv, Sk, Dh)), 'v_cache': _w((lambda *s: _rng.normal(s) * 0.05)(B, Hkv, Sk, Dh)), 'wq': _w((lambda *s: _rng.normal(s) * 0.05)(D, Hq * Dh) * D ** (-0.5)), 'wo': _w((lambda *s: _rng.normal(s) * 0.05)(Hq * Dh, D) * (Hq * Dh) ** (-0.5))}
    _A_in = _A_setup()

    def _B_setup():
        B, S, D, F = (1, 1, 448, 1792)
        return {'x': _w((lambda *s: _rng.normal(s) * 0.05)(B, S, D)), 'w1': _w((lambda *s: _rng.normal(s) * 0.05)(D, D) * D ** (-0.5)), 'w2': _w((lambda *s: _rng.normal(s) * 0.05)(D, D) * D ** (-0.5)), 'w3': _w((lambda *s: _rng.normal(s) * 0.05)(D, F) * D ** (-0.5)), 'w4': _w((lambda *s: _rng.normal(s) * 0.05)(F, D) * F ** (-0.5))}
    _B_in = _B_setup()
    return {'A_x': _A_in['x'], 'A_k_cache': _A_in['k_cache'], 'A_v_cache': _A_in['v_cache'], 'A_wq': _A_in['wq'], 'A_wo': _A_in['wo'], 'B_x': _B_in['x'], 'B_w1': _B_in['w1'], 'B_w2': _B_in['w2'], 'B_w3': _B_in['w3'], 'B_w4': _B_in['w4'], 'c': _w((lambda *s: _rng.normal(s) * 0.05)(1, 448)), 'w_mod': _w((lambda *s: _rng.normal(s) * 0.05)(448, 6 * 448) * 448 ** (-0.5))}

def reference(A_x, A_k_cache, A_v_cache, A_wq, A_wo, B_x, B_w1, B_w2, B_w3, B_w4, c, w_mod):

    def _A_ref(x, k_cache, v_cache, wq, wo):
        B, Sq, D = x.shape
        Hq, Dh = (16, 256)
        Hkv, Sk = (k_cache.shape[1], k_cache.shape[2])
        W = min(4096, max(256, Sk // 4))
        rep = Hq // Hkv
        q = (lambda x, *d: x.transpose(*d))((x @ wq).reshape(B, Sq, Hq, Dh), 0, 2, 1, 3)
        k = jnp.repeat(k_cache[:, :, Sk - W:, :], rep, axis=1)
        v = jnp.repeat(v_cache[:, :, Sk - W:, :], rep, axis=1)
        scores = jnp.einsum('bhqd,bhkd->bhqk', q, k) * Dh ** (-0.5)
        p = _softmax(scores, axis=-1)
        o = jnp.einsum('bhqk,bhkd->bhqd', p, v)
        return (lambda x, *d: x.transpose(*d))(o, 0, 2, 1, 3).reshape(B, Sq, Hq * Dh) @ wo

    def _B_ref(x, w1, w2, w3, w4):
        B, S, D = x.shape
        h = _gelu(_layernorm(x, axis=-1) @ w1)
        c = D // 4
        g0 = jnp.pad(h[:, :, 0 * c:1 * c], ((0, 0), (1, 0), (0, 0)))[:, :S, :]
        g1 = jnp.pad(h[:, :, 1 * c:2 * c], ((0, 0), (0, 1), (0, 0)))[:, 1:, :]
        g2 = jnp.pad(h[:, :, 2 * c:3 * c], ((0, 0), (2, 0), (0, 0)))[:, :S, :]
        g3 = jnp.pad(h[:, :, 3 * c:], ((0, 0), (0, 2), (0, 0)))[:, 2:, :]
        hs = jnp.concatenate([g0, g1, g2, g3], axis=-1) @ w2
        x1 = x + hs
        h2 = _gelu(_layernorm(x1, axis=-1) @ w3) @ w4
        return x1 + h2
    x = A_x
    mod = (_silu(c) @ w_mod).reshape(c.shape[0], 6, 1, -1)
    sa, ca, ga, sb, cb, gb = (mod[:, 0].copy(), mod[:, 1].copy(), mod[:, 2].copy(), mod[:, 3].copy(), mod[:, 4].copy(), mod[:, 5].copy())
    h = _layernorm(x, axis=-1) * (1 + ca) + sa
    x = x + ga * _A_ref(h, A_k_cache, A_v_cache, A_wq, A_wo)
    h = _layernorm(x, axis=-1) * (1 + cb) + sb
    x = x + gb * _B_ref(h, B_w1, B_w2, B_w3, B_w4)
    return x
```

```python
import jax
import jax.numpy as jnp
from jax import lax
import jax.experimental.pallas as pl
import jax.experimental.pallas.tpu as pltpu

HQ, DH = 16, 256
M = 8
BF = jnp.bfloat16
F32 = jnp.float32


def _nt(a, b):
    return lax.dot_general(a, b, (((1,), (1,)), ((), ())), preferred_element_type=F32)


def _nn(a, b):
    return jnp.dot(a, b, preferred_element_type=F32)


def _ln(x):
    m = jnp.mean(x, axis=-1, keepdims=True)
    d = x - m
    v = jnp.mean(d * d, axis=-1, keepdims=True)
    return d / jnp.sqrt(v + 1e-5)


def _kernel(x_hbm, k_hbm, v_hbm, wq_hbm, wo_hbm, w3_hbm, w4_hbm, c_hbm, wm_hbm, o_hbm,
            xb, cb_, kb, vb, wqb, wob, w3b, w4b, wmb, qs, ob, sems, ksem, vsem):
    SK = k_hbm.shape[2]
    HKV, W, _ = kb.shape
    D = xb.shape[1]
    cp = pltpu.make_async_copy
    d_wm = cp(wm_hbm, wmb, sems.at[0])
    d_c = cp(c_hbm, cb_, sems.at[1])
    d_x = cp(x_hbm.at[0], xb, sems.at[2])
    d_wq = cp(wq_hbm, wqb, sems.at[3])
    d_wo = cp(wo_hbm, wob, sems.at[4])
    d_w3 = cp(w3_hbm, w3b, sems.at[5])
    d_w4 = cp(w4_hbm, w4b, sems.at[6])
    d_o = cp(ob, o_hbm.at[0], sems.at[7])
    d_k = lambda h: cp(k_hbm.at[0, h, pl.ds(SK - W, W)], kb.at[h], ksem.at[h])
    d_v = lambda h: cp(v_hbm.at[0, h, pl.ds(SK - W, W)], vb.at[h], vsem.at[h])
    d_wm.start()
    d_c.start()
    d_x.start()
    d_wq.start()
    for h in range(HKV):
        d_k(h).start()
        d_v(h).start()
    d_wo.start()
    d_w3.start()
    d_w4.start()

    d_c.wait()
    d_x.wait()
    c = jnp.broadcast_to(cb_[...].astype(F32), (M, D))
    x = jnp.broadcast_to(xb[...].astype(F32), (M, D))
    sc = (c * jax.nn.sigmoid(c)).astype(BF)
    xn = _ln(x)
    d_wm.wait()
    mod = _nn(sc, wmb[...])
    sa, ca, ga, sb, cb, gb = (mod[:, i * D:(i + 1) * D] for i in range(6))
    h = (xn * (1.0 + ca) + sa).astype(BF)
    d_wq.wait()
    q = _nn(h, wqb[...]) * (DH ** -0.5)
    even = (lax.broadcasted_iota(jnp.int32, (M, DH), 0) & 1) == 0
    for j in range(HKV):
        qs[j] = jnp.where(even, q[:, 2 * j * DH:(2 * j + 1) * DH], q[:, (2 * j + 1) * DH:(2 * j + 2) * DH])

    def head(j, carry):
        d_k(j).wait()
        s = _nt(qs[j].astype(BF), kb[j])
        m = jnp.max(s, axis=-1, keepdims=True)
        p = jnp.exp(s - m)
        l = jnp.sum(p, axis=-1, keepdims=True)
        d_v(j).wait()
        o = _nn(p.astype(BF), vb[j])
        qs[j] = o / l
        return carry
    lax.fori_loop(0, HKV, head, 0)

    parts = []
    for j in range(HKV):
        o = qs[j]
        parts.append(jnp.where(even, o, 0.0))
        parts.append(jnp.where(even, 0.0, o))
    o = jnp.concatenate(parts, axis=1).astype(BF)
    d_wo.wait()
    a = _nt(o, wob[...])
    a = a + pltpu.roll(a, 1, 0)
    x = x + ga * a
    h = _ln(x) * (1.0 + cb) + sb
    hn = _ln(h).astype(BF)
    d_w3.wait()
    g = jax.nn.gelu(_nn(hn, w3b[...]), approximate=True).astype(BF)
    d_w4.wait()
    h2 = _nt(g, w4b[...])
    out = x + gb * (h + h2)
    ob[...] = out[0:1].astype(BF)
    d_o.start()
    d_o.wait()


@jax.jit
def pallas_adaLN_cond__sliding_block_cached__mixer_s_mlp__decode_kernel(
    A_x: jax.Array,
    A_k_cache: jax.Array,
    A_v_cache: jax.Array,
    A_wq: jax.Array,
    A_wo: jax.Array,
    B_x: jax.Array,
    B_w1: jax.Array,
    B_w2: jax.Array,
    B_w3: jax.Array,
    B_w4: jax.Array,
    c: jax.Array,
    w_mod: jax.Array,
):
    D = A_x.shape[-1]
    F = B_w3.shape[1]
    HKV, SK = A_k_cache.shape[1], A_k_cache.shape[2]
    W = min(4096, max(256, SK // 4))
    hbm = pl.BlockSpec(memory_space=pltpu.HBM)
    return pl.pallas_call(
        _kernel,
        out_shape=jax.ShapeDtypeStruct(A_x.shape, BF),
        in_specs=[hbm] * 9,
        out_specs=hbm,
        scratch_shapes=[
            pltpu.VMEM((1, D), BF), pltpu.VMEM((1, D), BF),
            pltpu.VMEM((HKV, W, DH), BF), pltpu.VMEM((HKV, W, DH), BF),
            pltpu.VMEM((D, HQ * DH), BF), pltpu.VMEM((D, HQ * DH), BF),
            pltpu.VMEM((D, F), BF), pltpu.VMEM((D, F), BF), pltpu.VMEM((D, 6 * D), BF),
            pltpu.VMEM((HKV, M, DH), F32), pltpu.VMEM((1, D), BF),
            pltpu.SemaphoreType.DMA((8,)), pltpu.SemaphoreType.DMA((HKV,)), pltpu.SemaphoreType.DMA((HKV,)),
        ],
        compiler_params=pltpu.CompilerParams(vmem_limit_bytes=100 << 20),
    )(A_x, A_k_cache, A_v_cache, A_wq, A_wo.T, B_w3, B_w4.T, c, w_mod)
```

```python
import jax
import jax.numpy as jnp
from jax import lax
import jax.experimental.pallas as pl
import jax.experimental.pallas.tpu as pltpu

HQ, DH = 16, 256
M = 8
LANES = 128
BF = jnp.bfloat16
F32 = jnp.float32

RING_SLOTS = (64, 56)
RING_CHUNKS = (64, 56, 32, 16)
W4_SPLIT = (256, 384)
GB_SPLIT = (352,)


def _nt(a, b):
    return lax.dot_general(a, b, (((1,), (1,)), ((), ())), preferred_element_type=F32)


def _nn(a, b):
    return jnp.dot(a, b, preferred_element_type=F32)


def _layernorm(x):
    d = x - jnp.mean(x, axis=-1, keepdims=True)
    return d / jnp.sqrt(jnp.mean(d * d, axis=-1, keepdims=True) + 1e-5)


def _pieces(split, end):
    edges = (0, *split, end)
    return list(zip(edges, edges[1:]))


def _kernel(x_hbm, k_hbm, v_hbm, wq_hbm, wo_hbm, w3_hbm, w4_hbm, c_hbm, wm_hbm, out_hbm,
            x_v, c_v, k_v, v_v, wq_v, wo_v, w3_v, w4_v, wm_v,
            head_v, p_v, l_v, s_col, row_v, out_v, sems, *slots):
    seq = k_hbm.shape[2]
    hkv, win, _ = k_v.shape
    d = x_v.shape[1]
    gb0 = pl.cdiv(5 * d, LANES) * LANES
    gb_cols = pl.ds(gb0, 6 * d - gb0)
    staged = sum(RING_CHUNKS)

    n_copies = [0]

    def copy(src, dst):
        n_copies[0] += 1
        return pltpu.make_async_copy(src, dst, sems.at[n_copies[0] - 1])

    cp_wm = copy(wm_hbm.at[:, pl.ds(0, gb0)], wm_v.at[:, pl.ds(0, gb0)])
    cp_c = copy(c_hbm, c_v)
    cp_x = copy(x_hbm.at[0], x_v)
    cp_wq = copy(wq_hbm, wq_v)
    cp_k = copy(k_hbm.at[0, :, pl.ds(seq - win, win)], k_v)
    cp_v = copy(v_hbm.at[0, :, pl.ds(seq - win, win)], v_v)
    cp_wo = copy(wo_hbm.at[pl.ds(staged, d - staged)], wo_v.at[pl.ds(staged, d - staged)])
    cp_w3 = copy(w3_hbm, w3_v)
    w4_rows = _pieces(W4_SPLIT, d)
    cp_w4 = [copy(w4_hbm.at[pl.ds(a, b - a)], w4_v.at[pl.ds(a, b - a)]) for a, b in w4_rows]
    gb_rows = _pieces(GB_SPLIT, d)
    cp_gb = [copy(wm_hbm.at[pl.ds(a, b - a), gb_cols], wm_v.at[pl.ds(a, b - a), gb_cols])
             for a, b in gb_rows]
    cp_out = copy(out_v, out_hbm.at[0])

    fills, drains, row = [], [], 0
    for i, rows in enumerate(RING_CHUNKS):
        slot = slots[i % len(slots)].at[pl.ds(0, rows)]
        fills.append(copy(wo_hbm.at[pl.ds(row, rows)], slot))
        drains.append(copy(slot, wo_v.at[pl.ds(row, rows)]))
        row += rows

    def ring_step(i):
        fills[i].wait()
        drains[i].start()
        if i >= 1 and i + 1 < len(fills):
            drains[i - 1].wait()
            fills[i + 1].start()

    cp_wm.start()
    fills[0].start()
    fills[1].start()
    for cp in (cp_c, cp_x, cp_wq, cp_k, cp_v, cp_wo, cp_w3, *cp_w4, *cp_gb):
        cp.start()

    cp_c.wait()
    cp_x.wait()
    c = jnp.broadcast_to(c_v[...].astype(F32), (M, d))
    x = jnp.broadcast_to(x_v[...].astype(F32), (M, d))
    s = (c * jax.nn.sigmoid(c)).astype(BF)
    s_pad = jnp.concatenate([s.astype(F32), jnp.zeros((M, s_col.shape[0] - d), F32)], axis=1)
    for t in range(0, s_col.shape[0], LANES):
        s_col[t:t + LANES, :] = jnp.broadcast_to(s_pad[0:1, t:t + LANES], (LANES, LANES)).T
    cp_wm.wait()
    mod = _nn(s, wm_v[:, 0:gb0])
    sa, ca, ga, sb, cb = (mod[:, i * d:(i + 1) * d] for i in range(5))
    row_v[0] = x
    row_v[1] = ga
    row_v[2] = sb
    row_v[3] = cb
    row_v[4, :, 0:gb0 - 5 * d] = mod[:, 5 * d:]
    h = (_layernorm(x) * (1.0 + ca) + sa).astype(BF)
    cp_wq.wait()
    q = _nn(h, wq_v[...]) * DH ** -0.5
    even = (lax.broadcasted_iota(jnp.int32, (M, DH), 0) & 1) == 0
    for j in range(hkv):
        head_v[j] = jnp.where(even, q[:, 2 * j * DH:(2 * j + 1) * DH],
                              q[:, (2 * j + 1) * DH:(2 * j + 2) * DH])

    ring_step(0)
    ring_step(1)

    def softmax_head(j, carry):
        scores = _nt(head_v[j].astype(BF), k_v[j])
        p = jnp.exp(scores - jnp.max(scores, axis=-1, keepdims=True))
        p_v[j] = p
        l_v[j] = jnp.broadcast_to(1.0 / jnp.sum(p, axis=-1, keepdims=True), (M, LANES))
        return carry

    cp_k.wait()
    lax.fori_loop(0, hkv, softmax_head, 0)

    ring_step(2)
    ring_step(3)

    def value_head(j, carry):
        o = _nn(p_v[j].astype(BF), v_v[j])
        head_v[j] = o * jnp.concatenate([l_v[j]] * (DH // LANES), axis=1)
        return carry

    cp_v.wait()
    lax.fori_loop(0, hkv, value_head, 0)

    parts = []
    for j in range(hkv):
        o = head_v[j]
        parts += [jnp.where(even, o, 0.0), jnp.where(even, 0.0, o)]
    o = jnp.concatenate(parts, axis=1).astype(BF)
    drains[2].wait()
    drains[3].wait()
    cp_wo.wait()
    attn = _nt(o, wo_v[...])
    attn = attn + pltpu.roll(attn, 1, 0)
    x = row_v[0] + row_v[1] * attn
    h = _layernorm(x) * (1.0 + row_v[3]) + row_v[2]
    hn = _layernorm(h).astype(BF)
    row_v[0] = x
    row_v[1] = h

    cp_w3.wait()
    g = jax.nn.gelu(_nn(hn, w3_v[...]), approximate=True).astype(BF)
    for cp, (a, b) in zip(cp_w4, w4_rows):
        cp.wait()
        row_v[1, :, a:b] = row_v[1, :, a:b] + _nt(g, w4_v[a:b, :])

    tiles = range(gb0, 6 * d, LANES)
    acc = [[None, None] for _ in tiles]
    for cp, (a, b) in zip(cp_gb, gb_rows):
        cp.wait()
        for n, r in enumerate(range(a, b, M)):
            s_blk = s_col[r:r + M, :]
            for j, t in enumerate(tiles):
                term = wm_v[r:r + M, t:t + LANES].astype(F32) * s_blk
                acc[j][n % 2] = term if acc[j][n % 2] is None else acc[j][n % 2] + term
    row_v[4, :, gb0 - 5 * d:d] = jnp.concatenate(
        [jnp.broadcast_to(jnp.sum(u + w, axis=0, keepdims=True), (M, LANES)) for u, w in acc],
        axis=1)

    out_v[...] = (row_v[0] + row_v[4] * row_v[1])[0:1].astype(BF)
    cp_out.start()
    cp_out.wait()


@jax.jit
def pallas_adaLN_cond__sliding_block_cached__mixer_s_mlp__decode_kernel(
    A_x: jax.Array,
    A_k_cache: jax.Array,
    A_v_cache: jax.Array,
    A_wq: jax.Array,
    A_wo: jax.Array,
    B_x: jax.Array,
    B_w1: jax.Array,
    B_w2: jax.Array,
    B_w3: jax.Array,
    B_w4: jax.Array,
    c: jax.Array,
    w_mod: jax.Array,
):
    assert A_x.shape[:2] == (1, 1)
    d = A_x.shape[-1]
    f = B_w3.shape[1]
    hkv, seq = A_k_cache.shape[1:3]
    win = min(4096, max(256, seq // 4))
    hbm = pl.BlockSpec(memory_space=pltpu.HBM)
    vmem = pltpu.VMEM
    return pl.pallas_call(
        _kernel,
        out_shape=jax.ShapeDtypeStruct(A_x.shape, BF),
        in_specs=[hbm] * 9,
        out_specs=hbm,
        scratch_shapes=[
            vmem((1, d), BF),
            vmem((1, d), BF),
            vmem((hkv, win, DH), BF),
            vmem((hkv, win, DH), BF),
            vmem((d, HQ * DH), BF),
            vmem((d, HQ * DH), BF),
            vmem((d, f), BF),
            vmem((d, f), BF),
            vmem((d, 6 * d), BF),
            vmem((hkv, M, DH), F32),
            vmem((hkv, M, win), F32),
            vmem((hkv, M, LANES), F32),
            vmem((pl.cdiv(d, LANES) * LANES, LANES), F32),
            vmem((5, M, d), F32),
            vmem((1, d), BF),
            pltpu.SemaphoreType.DMA((11 + len(W4_SPLIT) + len(GB_SPLIT) + 2 * len(RING_CHUNKS),)),
            *[pltpu.SMEM((rows, HQ * DH), BF) for rows in RING_SLOTS],
        ],
        compiler_params=pltpu.CompilerParams(
            vmem_limit_bytes=100 << 20, disable_semaphore_checks=True),
    )(A_x, A_k_cache, A_v_cache, A_wq, A_wo.T, B_w3, B_w4.T, c, w_mod)
```

```python
import jax
import jax.numpy as jnp
from jax import lax
import jax.experimental.pallas as pl
import jax.experimental.pallas.tpu as pltpu

HQ, DH = 16, 256
M = 8
LANES = 128
BF = jnp.bfloat16
F32 = jnp.float32

RING_SLOTS = (64, 56)
RING_CHUNKS = (64, 56, 32, 16)
W4_SPLIT = (256, 384)
GB_SPLIT = (288, 384)


def _nt(a, b):
    return lax.dot_general(a, b, (((1,), (1,)), ((), ())), preferred_element_type=F32)


def _nn(a, b):
    return jnp.dot(a, b, preferred_element_type=F32)


def _layernorm(x):
    d = x - jnp.mean(x, axis=-1, keepdims=True)
    return d / jnp.sqrt(jnp.mean(d * d, axis=-1, keepdims=True) + 1e-5)


def _pieces(split, end):
    edges = (0, *split, end)
    return list(zip(edges, edges[1:]))


def _kernel(x_hbm, k_hbm, v_hbm, wq_hbm, wo_hbm, w3_hbm, w4_hbm, c_hbm, wm_hbm, out_hbm,
            x_v, c_v, k_v, v_v, wq_v, wo_v, w3_v, w4_v, wm_v,
            head_v, p_v, l_v, s_col, row_v, gb_v, out_v, sems, *slots):
    seq = k_hbm.shape[2]
    hkv, win, _ = k_v.shape
    d = x_v.shape[1]
    gb0 = pl.cdiv(5 * d, LANES) * LANES
    gb_cols = pl.ds(gb0, 6 * d - gb0)
    staged = sum(RING_CHUNKS)

    n_copies = [0]

    def copy(src, dst):
        n_copies[0] += 1
        return pltpu.make_async_copy(src, dst, sems.at[n_copies[0] - 1])

    cp_wm = copy(wm_hbm.at[:, pl.ds(0, gb0)], wm_v.at[:, pl.ds(0, gb0)])
    cp_c = copy(c_hbm, c_v)
    cp_x = copy(x_hbm.at[0], x_v)
    cp_wq = copy(wq_hbm, wq_v)
    cp_k = copy(k_hbm.at[0, :, pl.ds(seq - win, win)], k_v)
    cp_v = copy(v_hbm.at[0, :, pl.ds(seq - win, win)], v_v)
    cp_wo = copy(wo_hbm.at[pl.ds(staged, d - staged)], wo_v.at[pl.ds(staged, d - staged)])
    cp_w3 = copy(w3_hbm, w3_v)
    w4_rows = _pieces(W4_SPLIT, d)
    cp_w4 = [copy(w4_hbm.at[pl.ds(a, b - a)], w4_v.at[pl.ds(a, b - a)]) for a, b in w4_rows]
    gb_rows = _pieces(GB_SPLIT, d)
    cp_gb = [copy(wm_hbm.at[pl.ds(a, b - a), gb_cols], wm_v.at[pl.ds(a, b - a), gb_cols])
             for a, b in gb_rows]
    cp_out = copy(out_v, out_hbm.at[0])

    fills, drains, row = [], [], 0
    for i, rows in enumerate(RING_CHUNKS):
        slot = slots[i % len(slots)].at[pl.ds(0, rows)]
        fills.append(copy(wo_hbm.at[pl.ds(row, rows)], slot))
        drains.append(copy(slot, wo_v.at[pl.ds(row, rows)]))
        row += rows

    def ring_step(i):
        fills[i].wait()
        drains[i].start()
        if i >= 1 and i + 1 < len(fills):
            drains[i - 1].wait()
            fills[i + 1].start()

    cp_wm.start()
    fills[0].start()
    fills[1].start()
    for cp in (cp_wq, cp_c, cp_x, cp_k, cp_v, cp_wo, cp_w3, *cp_w4, *cp_gb):
        cp.start()

    cp_c.wait()
    cp_x.wait()
    c = jnp.broadcast_to(c_v[...].astype(F32), (M, d))
    x = jnp.broadcast_to(x_v[...].astype(F32), (M, d))
    s = (c * jax.nn.sigmoid(c)).astype(BF)
    s_pad = jnp.concatenate([s.astype(F32), jnp.zeros((M, s_col.shape[0] - d), F32)], axis=1)
    for t in range(0, s_col.shape[0], LANES):
        s_col[t:t + LANES, :] = jnp.broadcast_to(s_pad[0:1, t:t + LANES], (LANES, LANES)).T
    cp_wm.wait()
    mod = _nn(s, wm_v[:, 0:gb0])
    sa, ca, ga, sb, cb = (mod[:, i * d:(i + 1) * d] for i in range(5))
    row_v[0] = x
    row_v[1] = ga
    row_v[2] = sb
    row_v[3] = cb
    lead = gb0 - 5 * d
    gb_v[...] = jnp.concatenate([mod[:, 5 * d:], jnp.zeros((M, LANES - lead), F32)], axis=1)
    h = (_layernorm(x) * (1.0 + ca) + sa).astype(BF)
    cp_wq.wait()
    q = _nn(h, wq_v[...]) * DH ** -0.5
    even = (lax.broadcasted_iota(jnp.int32, (M, DH), 0) & 1) == 0
    for j in range(hkv):
        head_v[j] = jnp.where(even, q[:, 2 * j * DH:(2 * j + 1) * DH],
                              q[:, (2 * j + 1) * DH:(2 * j + 2) * DH])

    ring_step(0)
    ring_step(1)

    def softmax_head(j, carry):
        scores = _nt(head_v[j].astype(BF), k_v[j])
        p = jnp.exp(scores - jnp.max(scores, axis=-1, keepdims=True))
        p_v[j] = p
        l_v[j] = jnp.broadcast_to(1.0 / jnp.sum(p, axis=-1, keepdims=True), (M, LANES))
        return carry

    cp_k.wait()
    lax.fori_loop(0, hkv, softmax_head, 0)

    ring_step(2)
    ring_step(3)

    def value_head(j, carry):
        o = _nn(p_v[j].astype(BF), v_v[j])
        head_v[j] = o * jnp.concatenate([l_v[j]] * (DH // LANES), axis=1)
        return carry

    cp_v.wait()
    lax.fori_loop(0, hkv, value_head, 0)

    parts = []
    for j in range(hkv):
        o = head_v[j]
        parts += [jnp.where(even, o, 0.0), jnp.where(even, 0.0, o)]
    o = jnp.concatenate(parts, axis=1).astype(BF)
    drains[2].wait()
    drains[3].wait()
    cp_wo.wait()
    attn = _nt(o, wo_v[...])
    attn = attn + pltpu.roll(attn, 1, 0)
    x = row_v[0] + row_v[1] * attn
    h = _layernorm(x) * (1.0 + row_v[3]) + row_v[2]
    hn = _layernorm(h).astype(BF)
    row_v[0] = x
    row_v[1] = h

    cp_w3.wait()
    g = jax.nn.gelu(_nn(hn, w3_v[...]), approximate=True).astype(BF)
    for cp, (a, b) in zip(cp_w4, w4_rows):
        cp.wait()
        row_v[1, :, a:b] = row_v[1, :, a:b] + _nt(g, w4_v[a:b, :])

    tiles = range(gb0, 6 * d, LANES)
    cols = [slice(t, min(t + LANES, d)) for t in range(0, d, LANES)]
    acc = [[None, None] for _ in tiles]
    for cp, (a, b) in zip(cp_gb, gb_rows):
        cp.wait()
        for n, r in enumerate(range(a, b, M)):
            s_blk = s_col[r:r + M, :]
            for j, t in enumerate(tiles):
                term = wm_v[r:r + M, t:t + LANES].astype(F32) * s_blk
                acc[j][n % 2] = term if acc[j][n % 2] is None else acc[j][n % 2] + term
    shifted = [gb_v[...]] + [
        pltpu.roll(jnp.broadcast_to(jnp.sum(u + w, axis=0, keepdims=True), (M, LANES)), lead, 1)
        for u, w in acc]
    low = lax.broadcasted_iota(jnp.int32, (M, LANES), 1) < lead
    out = []
    for i, col in enumerate(cols):
        gb = jnp.where(low, shifted[i], shifted[i + 1]) if i < len(tiles) else shifted[i]
        out.append(row_v[0, :, col] + gb[:, :col.stop - col.start] * row_v[1, :, col])
    out_v[...] = jnp.concatenate(out, axis=1)[0:1].astype(BF)
    cp_out.start()
    cp_out.wait()


@jax.jit
def pallas_adaLN_cond__sliding_block_cached__mixer_s_mlp__decode_kernel(
    A_x: jax.Array,
    A_k_cache: jax.Array,
    A_v_cache: jax.Array,
    A_wq: jax.Array,
    A_wo: jax.Array,
    B_x: jax.Array,
    B_w1: jax.Array,
    B_w2: jax.Array,
    B_w3: jax.Array,
    B_w4: jax.Array,
    c: jax.Array,
    w_mod: jax.Array,
):
    assert A_x.shape[:2] == (1, 1)
    d = A_x.shape[-1]
    f = B_w3.shape[1]
    hkv, seq = A_k_cache.shape[1:3]
    win = min(4096, max(256, seq // 4))
    hbm = pl.BlockSpec(memory_space=pltpu.HBM)
    vmem = pltpu.VMEM
    return pl.pallas_call(
        _kernel,
        out_shape=jax.ShapeDtypeStruct(A_x.shape, BF),
        in_specs=[hbm] * 9,
        out_specs=hbm,
        scratch_shapes=[
            vmem((1, d), BF),
            vmem((1, d), BF),
            vmem((hkv, win, DH), BF),
            vmem((hkv, win, DH), BF),
            vmem((d, HQ * DH), BF),
            vmem((d, HQ * DH), BF),
            vmem((d, f), BF),
            vmem((d, f), BF),
            vmem((d, 6 * d), BF),
            vmem((hkv, M, DH), F32),
            vmem((hkv, M, win), F32),
            vmem((hkv, M, LANES), F32),
            vmem((pl.cdiv(d, LANES) * LANES, LANES), F32),
            vmem((4, M, d), F32),
            vmem((M, LANES), F32),
            vmem((1, d), BF),
            pltpu.SemaphoreType.DMA((11 + len(W4_SPLIT) + len(GB_SPLIT) + 2 * len(RING_CHUNKS),)),
            *[pltpu.SMEM((rows, HQ * DH), BF) for rows in RING_SLOTS],
        ],
        compiler_params=pltpu.CompilerParams(
            vmem_limit_bytes=100 << 20, disable_semaphore_checks=True),
    )(A_x, A_k_cache, A_v_cache, A_wq, A_wo.T, B_w3, B_w4.T, c, w_mod)
```

```python
import jax
import jax.numpy as jnp
from jax import lax
import jax.experimental.pallas as pl
import jax.experimental.pallas.tpu as pltpu

HQ, DH = 16, 256
M = 8
LANES = 128
BF = jnp.bfloat16
F32 = jnp.float32

RING_SLOTS = (64, 56)
RING_CHUNKS = (64, 56, 32, 16)
W4_SPLIT = (256, 384)
GB_SPLIT = (288, 384)


def _nt(a, b):
    return lax.dot_general(a, b, (((1,), (1,)), ((), ())), preferred_element_type=F32)


def _nn(a, b):
    return jnp.dot(a, b, preferred_element_type=F32)


def _layernorm(x):
    d = x - jnp.mean(x, axis=-1, keepdims=True)
    return d / jnp.sqrt(jnp.mean(d * d, axis=-1, keepdims=True) + 1e-5)


def _pieces(split, end):
    edges = (0, *split, end)
    return list(zip(edges, edges[1:]))


def _kernel(x_hbm, k_hbm, v_hbm, wq_hbm, wo_hbm, w3_hbm, w4_hbm, c_hbm, wm_hbm, out_hbm,
            x_v, c_v, k_v, v_v, wq_v, wo_v, w3_v, w4_v, wm_v, wg_v,
            head_v, p_v, l_v, s_col, row_v, gb_v, out_v, sems, *slots):
    seq = k_hbm.shape[2]
    hkv, win, _ = k_v.shape
    d = x_v.shape[1]
    gb0 = wm_v.shape[1]
    staged = sum(RING_CHUNKS)

    n_copies = [0]

    def copy(src, dst):
        n_copies[0] += 1
        return pltpu.make_async_copy(src, dst, sems.at[n_copies[0] - 1])

    cp_wm = copy(wm_hbm.at[:, pl.ds(0, gb0)], wm_v)
    cp_c = copy(c_hbm, c_v)
    cp_x = copy(x_hbm.at[0], x_v)
    cp_wq = copy(wq_hbm, wq_v)
    cp_k = copy(k_hbm.at[0, :, pl.ds(seq - win, win)], k_v)
    cp_v = copy(v_hbm.at[0, :, pl.ds(seq - win, win)], v_v)
    cp_wo = copy(wo_hbm.at[pl.ds(staged, d - staged)], wo_v.at[pl.ds(staged, d - staged)])
    cp_w3 = copy(w3_hbm, w3_v)
    w4_rows = _pieces(W4_SPLIT, d)
    cp_w4 = [copy(w4_hbm.at[pl.ds(a, b - a)], w4_v.at[pl.ds(a, b - a)]) for a, b in w4_rows]
    gb_rows = _pieces(GB_SPLIT, d)
    cp_gb = [copy(wm_hbm.at[pl.ds(a, b - a), pl.ds(gb0, 6 * d - gb0)], wg_v.at[pl.ds(a, b - a)])
             for a, b in gb_rows]
    cp_out = copy(out_v, out_hbm.at[0])

    fills, drains, row = [], [], 0
    for i, rows in enumerate(RING_CHUNKS):
        slot = slots[i % len(slots)].at[pl.ds(0, rows)]
        fills.append(copy(wo_hbm.at[pl.ds(row, rows)], slot))
        drains.append(copy(slot, wo_v.at[pl.ds(row, rows)]))
        row += rows

    def ring_step(i):
        fills[i].wait()
        drains[i].start()
        if i >= 1 and i + 1 < len(fills):
            drains[i - 1].wait()
            fills[i + 1].start()

    cp_wm.start()
    fills[0].start()
    fills[1].start()
    for cp in (cp_wq, cp_c, cp_x, cp_k, cp_v, cp_wo, cp_w3, *cp_w4, *cp_gb):
        cp.start()

    cp_c.wait()
    cp_x.wait()
    c = jnp.broadcast_to(c_v[...].astype(F32), (M, d))
    x = jnp.broadcast_to(x_v[...].astype(F32), (M, d))
    s = (c * jax.nn.sigmoid(c)).astype(BF)
    s_pad = jnp.concatenate([s.astype(F32), jnp.zeros((M, s_col.shape[0] - d), F32)], axis=1)
    for t in range(0, s_col.shape[0], LANES):
        s_col[t:t + LANES, :] = jnp.broadcast_to(s_pad[0:1, t:t + LANES], (LANES, LANES)).T
    cp_wm.wait()
    mod = _nn(s, wm_v[...])
    sa, ca, ga, sb, cb = (mod[:, i * d:(i + 1) * d] for i in range(5))
    row_v[0] = x
    row_v[1] = ga
    row_v[2] = sb
    row_v[3] = cb
    lead = gb0 - 5 * d
    gb_v[...] = jnp.concatenate([mod[:, 5 * d:], jnp.zeros((M, LANES - lead), F32)], axis=1)
    h = (_layernorm(x) * (1.0 + ca) + sa).astype(BF)
    cp_wq.wait()
    q = _nn(h, wq_v[...]) * DH ** -0.5
    even = (lax.broadcasted_iota(jnp.int32, (M, DH), 0) & 1) == 0
    for j in range(hkv):
        head_v[j] = jnp.where(even, q[:, 2 * j * DH:(2 * j + 1) * DH],
                              q[:, (2 * j + 1) * DH:(2 * j + 2) * DH])

    ring_step(0)
    ring_step(1)

    def softmax_head(j, carry):
        scores = _nt(head_v[j].astype(BF), k_v[j])
        p = jnp.exp(scores - jnp.max(scores, axis=-1, keepdims=True))
        p_v[j] = p
        l_v[j] = jnp.broadcast_to(1.0 / jnp.sum(p, axis=-1, keepdims=True), (M, LANES))
        return carry

    cp_k.wait()
    lax.fori_loop(0, hkv, softmax_head, 0)

    ring_step(2)
    ring_step(3)

    def value_head(j, carry):
        o = _nn(p_v[j].astype(BF), v_v[j])
        head_v[j] = o * jnp.concatenate([l_v[j]] * (DH // LANES), axis=1)
        return carry

    cp_v.wait()
    lax.fori_loop(0, hkv, value_head, 0)

    parts = []
    for j in range(hkv):
        o = head_v[j]
        parts += [jnp.where(even, o, 0.0), jnp.where(even, 0.0, o)]
    o = jnp.concatenate(parts, axis=1).astype(BF)
    drains[2].wait()
    drains[3].wait()
    cp_wo.wait()
    attn = _nt(o, wo_v[...])
    attn = attn + pltpu.roll(attn, 1, 0)
    x = row_v[0] + row_v[1] * attn
    h = _layernorm(x) * (1.0 + row_v[3]) + row_v[2]
    hn = _layernorm(h).astype(BF)
    row_v[0] = x
    row_v[1] = h

    cp_w3.wait()
    g = jax.nn.gelu(_nn(hn, w3_v[...]), approximate=True).astype(BF)
    for cp, (a, b) in zip(cp_w4, w4_rows):
        cp.wait()
        row_v[1, :, a:b] = row_v[1, :, a:b] + _nt(g, w4_v[a:b, :])

    tiles = range(0, 6 * d - gb0, LANES)
    cols = [slice(t, min(t + LANES, d)) for t in range(0, d, LANES)]
    acc = [[None, None] for _ in tiles]
    for cp, (a, b) in zip(cp_gb, gb_rows):
        cp.wait()
        for n, r in enumerate(range(a, b, M)):
            s_blk = s_col[r:r + M, :]
            for j, t in enumerate(tiles):
                term = wg_v[r:r + M, t:t + LANES].astype(F32) * s_blk
                acc[j][n % 2] = term if acc[j][n % 2] is None else acc[j][n % 2] + term
    shifted = [gb_v[...]] + [
        pltpu.roll(jnp.broadcast_to(jnp.sum(u + w, axis=0, keepdims=True), (M, LANES)), lead, 1)
        for u, w in acc]
    low = lax.broadcasted_iota(jnp.int32, (M, LANES), 1) < lead
    out = []
    for i, col in enumerate(cols):
        gb = jnp.where(low, shifted[i], shifted[i + 1]) if i < len(tiles) else shifted[i]
        out.append(row_v[0, :, col] + gb[:, :col.stop - col.start] * row_v[1, :, col])
    out_v[...] = jnp.concatenate(out, axis=1)[0:1].astype(BF)
    cp_out.start()
    cp_out.wait()


@jax.jit
def pallas_adaLN_cond__sliding_block_cached__mixer_s_mlp__decode_kernel(
    A_x: jax.Array,
    A_k_cache: jax.Array,
    A_v_cache: jax.Array,
    A_wq: jax.Array,
    A_wo: jax.Array,
    B_x: jax.Array,
    B_w1: jax.Array,
    B_w2: jax.Array,
    B_w3: jax.Array,
    B_w4: jax.Array,
    c: jax.Array,
    w_mod: jax.Array,
):
    assert A_x.shape == (1, 1, 448)
    d = A_x.shape[-1]
    gb0 = pl.cdiv(5 * d, LANES) * LANES
    f = B_w3.shape[1]
    hkv, seq = A_k_cache.shape[1:3]
    win = min(4096, max(256, seq // 4))
    hbm = pl.BlockSpec(memory_space=pltpu.HBM)
    vmem = pltpu.VMEM
    return pl.pallas_call(
        _kernel,
        out_shape=jax.ShapeDtypeStruct(A_x.shape, BF),
        in_specs=[hbm] * 9,
        out_specs=hbm,
        scratch_shapes=[
            vmem((1, d), BF),
            vmem((1, d), BF),
            vmem((hkv, win, DH), BF),
            vmem((hkv, win, DH), BF),
            vmem((d, HQ * DH), BF),
            vmem((d, HQ * DH), BF),
            vmem((d, f), BF),
            vmem((d, f), BF),
            vmem((d, gb0), BF),
            vmem((d, 6 * d - gb0), BF),
            vmem((hkv, M, DH), F32),
            vmem((hkv, M, win), F32),
            vmem((hkv, M, LANES), F32),
            vmem((pl.cdiv(d, LANES) * LANES, LANES), F32),
            vmem((4, M, d), F32),
            vmem((M, LANES), F32),
            vmem((1, d), BF),
            pltpu.SemaphoreType.DMA((11 + len(W4_SPLIT) + len(GB_SPLIT) + 2 * len(RING_CHUNKS),)),
            *[pltpu.SMEM((rows, HQ * DH), BF) for rows in RING_SLOTS],
        ],
        compiler_params=pltpu.CompilerParams(
            vmem_limit_bytes=100 << 20, disable_semaphore_checks=True),
    )(A_x, A_k_cache, A_v_cache, A_wq, A_wo.T, B_w3, B_w4.T, c, w_mod)
```
